```python
import jax
import jax.numpy as jnp

def _softmax(x, axis=-1):
    return jax.nn.softmax(x, axis=axis)

def _gelu(x):
    return jax.nn.gelu(x, approximate=True)

def _silu(x):
    return jax.nn.silu(x)

def _sigmoid(x):
    return jax.nn.sigmoid(x)

def _layernorm(x, axis=-1, eps=1e-05):
    m = jnp.mean(x, axis=axis, keepdims=True)
    v = jnp.var(x, axis=axis, keepdims=True)
    return (x - m) / jnp.sqrt(v + eps)

def _scatter_add(tgt, idx, src, axis=0):
    return tgt.at[idx].add(src)

def _segment_sum(src, seg, n):
    return jax.ops.segment_sum(src, seg, n)

class _Rng:

    def __init__(self, key):
        self._k = key

    def _next(self):
        self._k, sub = jax.random.split(self._k)
        return sub

    def normal(self, shape):
        return jax.random.normal(self._next(), shape, dtype=jnp.bfloat16)

    def randint(self, lo, hi, shape):
        return jax.random.randint(self._next(), shape, lo, hi, dtype=jnp.int32)

    def uniform(self, shape, lo=0.0, hi=1.0):
        return jax.random.uniform(self._next(), shape, jnp.bfloat16, lo, hi)

    def permutation(self, n):
        return jax.random.permutation(self._next(), n)
kernel_name = 'concat_heads__memory_aug_recurrent_mem_tr__sliding_local_dilated__prompt'

def setup_inputs():
    _rng = _Rng(jax.random.key(int.from_bytes(__import__("os").urandom(4), "little")))
    _w = lambda a: (lambda t: t.astype(jnp.bfloat16) if jnp.issubdtype(t.dtype, jnp.floating) else t)(jnp.asarray(a))

    def _A_setup():
        B, S, Dm = (1, 2048, 1024)
        H, Dh = (32, 128)
        M, seg = (8, 32)
        seg = min(seg, S)
        S = S // seg * seg
        return {'x': _w((lambda *s: _rng.normal(s) * 0.05)(B, S, Dm)), 'mem0': _w((lambda *s: _rng.normal(s) * 0.05)(B, M, Dm)), 'Wq': _w((lambda *s: _rng.normal(s) * 0.05)(Dm, H, Dh) * Dm ** (-0.5)), 'Wk': _w((lambda *s: _rng.normal(s) * 0.05)(Dm, H, Dh) * Dm ** (-0.5)), 'Wv': _w((lambda *s: _rng.normal(s) * 0.05)(Dm, H, Dh) * Dm ** (-0.5)), 'Wo': _w((lambda *s: _rng.normal(s) * 0.05)(H, Dh, Dm) * (H * Dh) ** (-0.5)), 'seg_len': seg}
    _A_in = _A_setup()

    def _B_setup():
        B, S, D = (1, 2048, 1024)
        return {'x': _w((lambda *s: _rng.normal(s) * 0.05)(B, S, D)), 'wqkv': _w((lambda *s: _rng.normal(s) * 0.05)(D, 3 * D)), 'wo': _w((lambda *s: _rng.normal(s) * 0.05)(D, D))}
    _B_in = _B_setup()
    return {'A_x': _A_in['x'], 'A_mem0': _A_in['mem0'], 'A_Wq': _A_in['Wq'], 'A_Wk': _A_in['Wk'], 'A_Wv': _A_in['Wv'], 'A_Wo': _A_in['Wo'], 'A_seg_len': _A_in['seg_len'], 'B_x': _B_in['x'], 'B_wqkv': _B_in['wqkv'], 'B_wo': _B_in['wo']}

def reference(A_x, A_mem0, A_Wq, A_Wk, A_Wv, A_Wo, A_seg_len, B_x, B_wqkv, B_wo):

    def _A_ref(x, mem0, Wq, Wk, Wv, Wo, seg_len):
        B, S, Dm = x.shape
        H, Dh = (Wq.shape[1], Wq.shape[2])
        M = mem0.shape[1]
        scale = Dh ** (-0.5)
        n_seg = S // seg_len
        L = M + seg_len
        idx = jnp.arange(L)
        mask = (idx[:, None] < M) | (idx[:, None] >= idx[None, :])
        mem = mem0
        outs = []
        for s in range(n_seg):
            xs = x[:, s * seg_len:(s + 1) * seg_len, :].copy()
            h = jnp.concatenate([mem, xs], axis=1)
            q = jnp.einsum('btd,dhe->bhte', h, Wq)
            k = jnp.einsum('btd,dhe->bhte', h, Wk)
            v = jnp.einsum('btd,dhe->bhte', h, Wv)
            scores = jnp.einsum('bhqe,bhke->bhqk', q, k) * scale
            scores = jnp.where(mask[None, None], scores, -1000000000.0)
            p = _softmax(scores, axis=-1)
            o = jnp.einsum('bhqk,bhke->bhqe', p, v)
            o = jnp.einsum('bhte,hed->btd', o, Wo)
            mem = o[:, :M, :].copy()
            outs.append(o[:, M:, :])
        return jnp.concatenate(outs, axis=1)

    def _B_ref(x, wqkv, wo):
        B, S, D = x.shape
        H = 32
        Dh = D // H
        W, dil = (8, 2)
        qkv = (lambda x, *d: x.transpose(*d))((x @ wqkv).reshape(B, S, 3, H, Dh), 2, 0, 3, 1, 4)
        q, k, v = (qkv[0], qkv[1], qkv[2])
        scale = Dh ** (-0.5)
        pos = jnp.arange(S)
        off = jnp.arange(W) * dil
        idx = pos[:, None] - off[None, :]
        mask = idx >= 0
        idx_c = jnp.where(mask, idx, 0).reshape(-1)
        kg = k[:, :, idx_c, :].reshape(B, H, S, W, Dh)
        vg = v[:, :, idx_c, :].reshape(B, H, S, W, Dh)
        logits = jnp.einsum('bhsd,bhswd->bhsw', q, kg) * scale
        logits = jnp.where(mask[None, None, :, :], logits, -1000000000.0)
        attn = _softmax(logits, axis=-1)
        o = jnp.einsum('bhsw,bhswd->bhsd', attn, vg)
        return (lambda x, *d: x.transpose(*d))(o, 0, 2, 1, 3).reshape(B, S, D) @ wo
    a = _A_ref(A_x, A_mem0, A_Wq, A_Wk, A_Wv, A_Wo, A_seg_len)
    b = _B_ref(B_x, B_wqkv, B_wo)
    return jnp.concatenate([a, b], axis=-1)
```

```python
import numpy as np
import jax
import jax.numpy as jnp
from jax import lax
import jax.experimental.pallas as pl
import jax.experimental.pallas.tpu as pltpu

F32, BF16, U32 = jnp.float32, jnp.bfloat16, jnp.uint32

S = 2048
D = 1024
HA, DHA = 32, 128
NMEM, SEG = 8, 32
HB, DHB = 32, 32
WIN, DIL = 8, 2
HALO = 16
NEG = -1000000000.0

RB = 512
NRB = S // RB
DC = 32
NDC = D // DC


def _bf16_rows(words):
    return pltpu.bitcast(words, BF16)


def _dot(a, b):
    return jnp.dot(a, b, preferred_element_type=F32)


def _kernel(xa_hbm, mem0_ref, wq_hbm, wk_hbm, wv_hbm, wo_hbm, xb_hbm, wqkvb_hbm, wob_hbm,
            out_hbm,
            wa, wo, wb, wob, rawa, rawb, rawob, qkvb, xa, xb, ostage,
            sem_xb, sem_wb, sem_a, sem_misc, sem_out):

    def xb_copy(r):
        rows = pl.ds(pl.multiple_of(r * RB, RB), RB)
        return pltpu.make_async_copy(xb_hbm.at[rows], xb.at[rows], sem_xb.at[r])

    def wqb_copy():
        cols = pl.ds(0, D)
        return pltpu.make_async_copy(wqkvb_hbm.at[:, cols], rawb.at[:, cols], sem_misc.at[0])

    def wkvb_copy(r):
        rows = pl.ds(pl.multiple_of(r * (D // NRB), D // NRB), D // NRB)
        cols = pl.ds(D, 2 * D)
        return pltpu.make_async_copy(wqkvb_hbm.at[rows, cols], rawb.at[rows, cols], sem_wb.at[r])

    def a_copies(c):
        return [pltpu.make_async_copy(w.at[c], rawa.at[m, c], sem_a.at[c])
                for m, w in enumerate((wq_hbm, wk_hbm, wv_hbm))]

    def wo_copy(n):
        return pltpu.make_async_copy(
            wo_hbm.at[:, pl.ds(n * 128, 128)], wo.at[n], sem_misc.at[1])

    def wob_copy(n):
        return pltpu.make_async_copy(
            wob_hbm.at[:, pl.ds(n * 128, 128)], rawob.at[n], sem_misc.at[2])

    def xa_copy():
        return pltpu.make_async_copy(xa_hbm, xa, sem_misc.at[3])

    def out_copy(i, slot):
        rows = pl.ds(pl.multiple_of(i * 2 * SEG, 2 * SEG), 2 * SEG)
        return pltpu.make_async_copy(ostage.at[slot], out_hbm.at[rows], sem_out.at[slot])

    def permute_b_cols(chunk, row0, nrows):
        raw = rawb[pl.ds(pl.multiple_of(2 * row0, 16), 2 * nrows), chunk * D:(chunk + 1) * D]
        words = pltpu.bitcast(raw, U32)
        t = [words[:, g * 128:(g + 1) * 128] for g in range(8)]
        lane = lax.broadcasted_iota(jnp.int32, (nrows, 128), 1)
        for bit in (1, 2, 4):
            low = (lane & (2 * bit)) == 0
            for g in range(8):
                if not g & bit:
                    x, y = t[g], t[g | bit]
                    t[g] = jnp.where(low, x, pltpu.roll(y, 2 * bit, 1))
                    t[g | bit] = jnp.where(low, pltpu.roll(x, 128 - 2 * bit, 1), y)
        for g in range(8):
            wb[chunk, pl.ds(pl.multiple_of(row0, 8), nrows), g * 128:(g + 1) * 128] = t[g]

    def permute_b_out_rows(n):
        src = rawob.bitcast(U32)
        for u in range(D // 16):
            wob[u * 8:(u + 1) * 8, n * 128:(n + 1) * 128] = (
                src[n, pl.ds((u & 7) * 8 + (u >> 3), 8, stride=64), :])

    def repack_a(c):
        src = rawa.bitcast(U32)
        for t in range(DC // 16):
            rows = pl.ds(pl.multiple_of(c * (DC // 2) + t * 8, 8), 8)
            for m in range(3):
                for hp in range(HA // 2):
                    even = src[m, c, pl.ds(t * 256 + hp, 8, stride=32), :]
                    odd = src[m, c, pl.ds(t * 256 + 16 + hp, 8, stride=32), :]
                    c0 = (2 * hp * 3 + m) * 128
                    c1 = c0 + 3 * 128
                    wa[rows, c0:c0 + 128] = (even & np.uint32(0xFFFF)) | (odd << 16)
                    wa[rows, c1:c1 + 128] = (even >> 16) | (odd & np.uint32(0xFFFF0000))

    def project_b(chunk, r):
        rows = pl.ds(pl.multiple_of(r * RB, RB), RB)
        y = _dot(xb[rows, :], _bf16_rows(wb[chunk]))
        for j in range(8):
            qkvb[chunk * 8 + j, pl.ds(pl.multiple_of(HALO + r * RB, 8), RB), :] = (
                y[:, j * 128:(j + 1) * 128])

    wqb_copy().start()
    xb_copy(0).start()
    wqb_copy().wait()
    wkvb_copy(0).start()
    xb_copy(1).start()
    permute_b_cols(0, 0, D // 2)

    a_per_step = NDC // (4 * NRB)

    def q_step(r, carry):
        @pl.when(r + 1 < NRB)
        def _():
            wkvb_copy(r + 1).start()

        @pl.when(r + 2 < NRB)
        def _():
            xb_copy(r + 2).start()

        for t in range(a_per_step):
            for cp in a_copies(r * a_per_step + t):
                cp.start()
        xb_copy(r).wait()
        wkvb_copy(r).wait()
        project_b(0, r)
        for chunk in (1, 2):
            permute_b_cols(chunk, r * (D // 2 // NRB), D // 2 // NRB)
        return carry

    lax.fori_loop(0, NRB, q_step, 0)

    def k_step(r, carry):
        for t in range(3 * a_per_step):
            for cp in a_copies(NRB * a_per_step + r * 3 * a_per_step + t):
                cp.start()
        for t in range(2 * a_per_step):
            for cp in a_copies(r * 2 * a_per_step + t):
                cp.wait()
        project_b(1, r)
        for t in range(2 * a_per_step):
            repack_a(r * 2 * a_per_step + t)
        return carry

    lax.fori_loop(0, NRB, k_step, 0)

    def v_step(r, carry):
        for n in range(8):
            @pl.when(r == n * NRB // 8)
            def _():
                wob_copy(n).start()
                wo_copy(n).start()

        @pl.when(r == 0)
        def _():
            xa_copy().start()

        for t in range(2 * a_per_step):
            for cp in a_copies((NRB + r) * 2 * a_per_step + t):
                cp.wait()
        project_b(2, r)
        for t in range(2 * a_per_step):
            repack_a((NRB + r) * 2 * a_per_step + t)
        return carry

    lax.fori_loop(0, NRB, v_step, 0)

    for j in range(8, 24):
        qkvb[j, 0:HALO, :] = jnp.broadcast_to(qkvb[j, HALO:HALO + 1, :], (HALO, 128))

    for n in range(8):
        wob_copy(n).wait()
    for n in range(8):
        permute_b_out_rows(n)
    for n in range(8):
        wo_copy(n).wait()
    xa_copy().wait()

    L = NMEM + SEG
    row = lax.broadcasted_iota(jnp.int32, (2 * L, 2 * L), 0)
    col = lax.broadcasted_iota(jnp.int32, (2 * L, 2 * L), 1)
    same_head = (row < L) == (col < L)
    row = jnp.where(row < L, row, row - L)
    col = jnp.where(col < L, col, col - L)
    visible = same_head & ((row < NMEM) | (row >= col))
    hidden = jnp.where(same_head, NEG, -jnp.inf).astype(F32)
    wo_words = wo.bitcast(U32)

    def a_project(h, g):
        out = []
        for hh in range(8 * g, 8 * g + 8):
            out.append(_dot(h, _bf16_rows(wa[:, hh * 384:(hh + 1) * 384])))
        return out

    def a_scores(heads):
        out = []
        for p in range(0, 8, 2):
            y = jnp.concatenate(heads[p:p + 2], axis=0).astype(BF16)
            s = lax.dot_general(y[:, 0:128], y[:, 128:256], (((1,), (1,)), ((), ())),
                                preferred_element_type=F32)
            out.append((s, y[:, 256:384]))
        return out

    def a_values(scored):
        out = []
        for s, v in scored:
            s = jnp.where(visible, s * DHA ** -0.5, hidden)
            e = jnp.exp(s - jnp.max(s, axis=-1, keepdims=True))
            o = _dot(e.astype(BF16), v) * (1.0 / jnp.sum(e, axis=-1, keepdims=True))
            out += [o[:L], o[L:]]
        return out

    def a_output(o, g):
        lhs = jnp.concatenate(o, axis=1).astype(BF16)
        w = jnp.concatenate(
            [_bf16_rows(wo_words[n, g * 512:(g + 1) * 512, :]) for n in range(8)], axis=1)
        return _dot(lhs, w)

    def a_segment(h, pick_rows, out_rows, filler):
        y, s, o, acc = [None] * 4, [None] * 4, [None] * 4, None

        def attend(g):
            s[g] = a_scores([pick_rows(8 * g + k, y[g][k]) for k in range(8)])

        def emit(g):
            part = a_output([out_rows(8 * g + k, o[g][k]) for k in range(8)], g)
            return part if acc is None else acc + part

        y[0] = a_project(h, 0)
        y[1] = a_project(h, 1)
        attend(0)
        y[2] = a_project(h, 2)
        o[0] = a_values(s[0])
        attend(1)
        y[3] = a_project(h, 3)
        o[1] = a_values(s[1])
        attend(2)
        acc = emit(0)
        attend(3)
        o[2] = a_values(s[2])
        acc = emit(1)
        o[3] = a_values(s[3])
        acc = emit(2)
        acc = emit(3)
        filler()
        return sum(y, []), sum(o, []), acc

    def b_attention(t0):
        base = pl.ds(pl.multiple_of(t0, SEG), HALO + SEG)
        lane = lax.broadcasted_iota(jnp.int32, (SEG, 128), 1)
        pos = lax.broadcasted_iota(jnp.int32, (SEG, 128), 0) + t0

        def window(j, w):
            return qkvb.at[j, base][HALO - w * DIL:HALO - w * DIL + SEG, :]

        def exchange_sum(x, v):
            return x + jnp.where((lane & v) == 0, pltpu.roll(x, 128 - v, 1), pltpu.roll(x, v, 1))

        q = [window(j, 0) for j in range(8)]
        logits = []
        for w in range(WIN):
            acc = q[0] * window(8, w)
            for j in range(1, 8):
                acc = acc + q[j] * window(8 + j, w)
            acc = exchange_sum(exchange_sum(acc, 16), 1) * DHB ** -0.5
            logits.append(jnp.where(pos >= w * DIL, acc, NEG) if w else acc)
        top = logits[0]
        for x in logits[1:]:
            top = jnp.maximum(top, x)
        e = [jnp.exp(x - top) for x in logits]
        total = e[0]
        for x in e[1:]:
            total = total + x
        inv = 1.0 / total
        p = [x * inv for x in e]
        out = []
        for j in range(8):
            acc = p[0] * window(16 + j, 0)
            for w in range(1, WIN):
                acc = acc + p[w] * window(16 + j, w)
            out.append(acc)
        return jnp.concatenate(out, axis=1).astype(BF16)

    def two_segments(i, mem):
        slot = i % 2

        @pl.when(i >= 2)
        def _():
            out_copy(i - 2, slot).wait()

        def b_block(k):
            def run():
                o = b_attention(i * 2 * SEG + k * SEG)
                ostage[slot, k * SEG:(k + 1) * SEG, D:2 * D] = (
                    _dot(o, _bf16_rows(wob[...])).astype(BF16))
            return run

        x = xa[pl.ds(pl.multiple_of(i * 2 * SEG, 2 * SEG), 2 * SEG), :].astype(F32)

        h = jnp.concatenate([mem, x[:SEG + 8]], axis=0).astype(BF16)
        y0, o0, out0 = a_segment(
            h, lambda hh, y: y[:L], lambda hh, o: o[:L - 8], b_block(0))
        ostage[slot, 0:SEG - 8, 0:D] = out0[NMEM:].astype(BF16)

        h = jnp.concatenate([out0[:NMEM], x[SEG + 8:]], axis=0).astype(BF16)
        _, _, out1 = a_segment(
            h,
            lambda hh, y: jnp.concatenate([y[:NMEM], y0[hh][L:], y[NMEM:]], axis=0),
            lambda hh, o: jnp.concatenate([o[:NMEM], o0[hh][L - 8:], o[NMEM:]], axis=0),
            b_block(1))
        ostage[slot, SEG - 8:2 * SEG, 0:D] = out1[NMEM:].astype(BF16)

        out_copy(i, slot).start()
        return out1[:NMEM]

    steps = S // (2 * SEG)
    lax.fori_loop(0, steps, two_segments, mem0_ref[...].astype(F32))
    for i in (steps - 2, steps - 1):
        out_copy(i, i % 2).wait()


def pallas_concat_heads__memory_aug_recurrent_mem_tr__sliding_local_dilated__prompt_kernel(
    A_x, A_mem0, A_Wq, A_Wk, A_Wv, A_Wo, A_seg_len, B_x, B_wqkv, B_wo,
):
    assert A_seg_len == SEG and A_x.shape == (1, S, D) and A_mem0.shape == (1, NMEM, D)
    assert A_Wq.shape == (D, HA, DHA) and B_x.shape == (1, S, D)
    hbm = pl.BlockSpec(memory_space=pl.ANY)
    chunked = (NDC, DC * HA, DHA)
    out = pl.pallas_call(
        _kernel,
        out_shape=jax.ShapeDtypeStruct((S, 2 * D), BF16),
        in_specs=[hbm, pl.BlockSpec(memory_space=pltpu.VMEM)] + [hbm] * 7,
        out_specs=hbm,
        scratch_shapes=[
            pltpu.VMEM((D // 2, 3 * HA * DHA), U32),
            pltpu.VMEM((8, HA * DHA, 128), BF16),
            pltpu.VMEM((3, D // 2, D), U32),
            pltpu.VMEM((D // 2, D), U32),
            pltpu.VMEM((3,) + chunked, BF16),
            pltpu.VMEM((D, 3 * D), BF16),
            pltpu.VMEM((8, D, 128), BF16),
            pltpu.VMEM((24, HALO + S, 128), F32),
            pltpu.VMEM((S, D), BF16),
            pltpu.VMEM((S, D), BF16),
            pltpu.VMEM((2, 2 * SEG, 2 * D), BF16),
            pltpu.SemaphoreType.DMA((NRB,)),
            pltpu.SemaphoreType.DMA((NRB,)),
            pltpu.SemaphoreType.DMA((NDC,)),
            pltpu.SemaphoreType.DMA((4,)),
            pltpu.SemaphoreType.DMA((2,)),
        ],
        compiler_params=pltpu.CompilerParams(vmem_limit_bytes=120 * 1024 * 1024),
    )(
        A_x.reshape(S, D), A_mem0.reshape(NMEM, D),
        A_Wq.reshape(chunked), A_Wk.reshape(chunked), A_Wv.reshape(chunked),
        A_Wo.reshape(HA * DHA, D),
        B_x.reshape(S, D), B_wqkv, B_wo,
    )
    return out.reshape(1, S, 2 * D)
```

```python
import functools

import numpy as np
import jax
import jax.numpy as jnp
from jax import lax
import jax.experimental.pallas as pl
import jax.experimental.pallas.tpu as pltpu

F32, BF16, U32 = jnp.float32, jnp.bfloat16, jnp.uint32

S = 2048
D = 1024
HA, DHA = 32, 128
NMEM, SEG = 8, 32
HB, DHB = 32, 32
WIN, DIL = 8, 2
HALO = 16
NEG = -1000000000.0
LOG2E = float(np.log2(np.e))

RB = 512
RP = 128
ROWS = 2 * SEG
XA_HEAD = 256
KC = 128
PITCH_A = D // 2 + 1
PITCH_B = 64 + 1


def _bf16_rows(words):
    return pltpu.bitcast(words, BF16)


def _dot(a, b):
    return jnp.dot(a, b, preferred_element_type=F32)


def _reciprocal(x):
    r = pl.reciprocal(x, approx=True)
    return r * (2.0 - x * r)


def _kernel(zero, xa_hbm, mem0_ref, wq_hbm, wk_hbm, wv_hbm, wo_hbm, xb_hbm, wqkvb_hbm, wob_hbm,
            out_hbm,
            wa, wo, wb, wob, rawa, rawb, rawob, qkvb, xa, xb, ostage, accum,
            sem_in, sem_out):

    def part(src, dst, *idx):
        return src.at[idx], dst.at[idx]

    def a_weights(lo, hi):
        return [(w.at[lo:hi], rawa.at[m, lo:hi]) for m, w in enumerate((wq_hbm, wk_hbm, wv_hbm))]

    def panels(src, dst):
        return [(src.at[:, n * 128:(n + 1) * 128], dst.at[n]) for n in range(D // 128)]

    every = slice(None)
    k_slices = [slice(c * KC, (c + 1) * KC) for c in range(D // KC)]
    wq_b = [part(wqkvb_hbm, rawb, ks, slice(0, D)) for ks in k_slices]
    x_b = [part(xb_hbm, xb, slice(0, RB), ks) for ks in k_slices]
    batches = [wq_b[:1]] + [list(pair) for pair in zip(wq_b[1:], x_b)] + [
        x_b[-1:],
        [part(xb_hbm, xb, slice(RB, 3 * RB))],
        [part(xb_hbm, xb, slice(3 * RB, S)), part(wqkvb_hbm, rawb, every, slice(D, 3 * D))],
        a_weights(0, 24),
        a_weights(24, 56),
        a_weights(56, 64) + panels(wob_hbm, rawob),
        panels(wo_hbm, wo) + [part(xa_hbm, xa, slice(0, XA_HEAD))],
        [part(xa_hbm, xa, slice(XA_HEAD, S))],
    ]
    batches = [[pltpu.make_async_copy(src, dst, sem_in.at[n]) for src, dst in batch]
               for n, batch in enumerate(batches)]
    pending = iter(batches)

    def wait_next_batch():
        for copy in next(pending):
            copy.wait()

    def out_copy(i, slot):
        rows = pl.ds(pl.multiple_of(i * ROWS, ROWS), ROWS)
        return pltpu.make_async_copy(ostage.at[slot], out_hbm.at[rows], sem_out.at[slot])

    def permute_b_cols(chunk, row0, nrows):
        words = pltpu.bitcast(rawb[2 * row0:2 * (row0 + nrows), chunk * D:(chunk + 1) * D], U32)
        t = [words[:, g * 128:(g + 1) * 128] for g in range(8)]
        lane = lax.broadcasted_iota(jnp.int32, (nrows, 128), 1)
        for bit in (1, 2, 4):
            low = (lane & (2 * bit)) == 0
            for g in range(8):
                if not g & bit:
                    x, y = t[g], t[g | bit]
                    t[g] = jnp.where(low, x, pltpu.roll(y, 2 * bit, 1))
                    t[g | bit] = jnp.where(low, pltpu.roll(x, 128 - 2 * bit, 1), y)
        for g in range(8):
            wb[chunk, row0:row0 + nrows, g * 128:(g + 1) * 128] = t[g]

    def permute_b_out_rows(n, half, zeros):
        src = rawob.bitcast(U32)
        for a in range(32 * half, 32 * half + 32):
            start = n * 8 * PITCH_B + (a & 7) * 8 + (a >> 3)
            wob[pl.ds(start, 8, stride=PITCH_B), :] = src[n, a * 8:(a + 1) * 8, :] | zeros

    def repack_a(t, m, zeros):
        src = rawa.bitcast(U32)
        half_word = zeros | 16
        for i in range(8):
            for half in range(2):
                r = 32 * i + 8 * half
                even, odd = src[m, t, r:r + 8, :], src[m, t, r + 16:r + 24, :]
                start = (m * HA + 8 * half) * PITCH_A + 8 * t + i
                wa[pl.ds(start, 8, stride=PITCH_A), :] = (
                    (even & np.uint32(0xFFFF)) | (odd << half_word))
                wa[pl.ds(start + HA // 2 * PITCH_A, 8, stride=PITCH_A), :] = (
                    (even >> half_word) | (odd & np.uint32(0xFFFF0000)))

    def repack_jobs(lo, hi):
        return [functools.partial(repack_a, t, m) for t in range(lo, hi) for m in range(3)]

    def a_weight(m, head):
        start = (m * HA + (head % 2) * (HA // 2) + head // 2) * PITCH_A
        return _bf16_rows(wa[start:start + D // 2, :])

    def project_b(chunk, r, side_jobs=()):
        y = _dot(xb[r * RP:(r + 1) * RP, :], _bf16_rows(wb[chunk]))
        for j in range(8):
            qkvb[chunk * 8 + j, HALO + r * RP:HALO + (r + 1) * RP, :] = y[:, j * 128:(j + 1) * 128]
        for k, job in enumerate(side_jobs):
            j, i = divmod(k * RP // len(side_jobs), RP // 8)
            done = y[8 * i:8 * i + 8, j * 128:(j + 1) * 128]
            job(pltpu.bitcast(done, U32) & zero[0].astype(U32))

    for batch in batches:
        for copy in batch:
            copy.start()

    wait_next_batch()
    permute_b_cols(0, 0, KC // 2)
    for c in range(D // KC):
        wait_next_batch()
        for r in range(RB // RP):
            rows = slice(HALO + r * RP, HALO + (r + 1) * RP)
            y = _dot(xb[r * RP:(r + 1) * RP, c * KC:(c + 1) * KC],
                     _bf16_rows(wb[0, c * KC // 2:(c + 1) * KC // 2, :]))
            for j in range(8):
                piece = y[:, j * 128:(j + 1) * 128]
                qkvb[j, rows, :] = piece + qkvb[j, rows, :] if c else piece
        if c + 1 < D // KC:
            permute_b_cols(0, (c + 1) * KC // 2, KC // 2)

    wait_next_batch()
    for r in range(4, 12):
        project_b(0, r)
    wait_next_batch()
    for r in range(4):
        project_b(0, 12 + r)
        permute_b_cols(1, r * D // 8, D // 8)
    for r in range(4):
        project_b(1, r)
        permute_b_cols(2, r * D // 8, D // 8)
    wait_next_batch()
    for r in range(12):
        project_b(1, 4 + r, repack_jobs(2 * r, 2 * r + 2))
    wait_next_batch()
    for r in range(8):
        project_b(2, r, repack_jobs(24 + 4 * r, 28 + 4 * r))
    wait_next_batch()
    for r in range(8):
        project_b(2, 8 + r, repack_jobs(56 + r, 57 + r)
                  + [functools.partial(permute_b_out_rows, r, half) for half in range(2)])

    for j in range(8, 24):
        qkvb[j, 0:HALO, :] = jnp.broadcast_to(qkvb[j, HALO:HALO + 1, :], (HALO, 128))
    wait_next_batch()

    L = NMEM + SEG
    row = lax.broadcasted_iota(jnp.int32, (2 * L, 128), 0)
    col = lax.broadcasted_iota(jnp.int32, (2 * L, 128), 1)
    same_head = ((row < L) == (col < L)) & (col < 2 * L)
    row = jnp.where(row < L, row, row - L)
    col = jnp.where(col < L, col, col - L)
    visible = same_head & ((row < NMEM) | (row >= col))
    gain = jnp.where(visible, DHA ** -0.5 * LOG2E, 0.0).astype(F32)
    bias = jnp.where(visible, 0.0, jnp.where(same_head, NEG * LOG2E, -jnp.inf)).astype(F32)
    wo_words = wo.bitcast(U32)
    pad = jnp.zeros((128 - 2 * L, 128), F32)

    def a_project(h, g):
        out = []
        for hh in range(8 * g, 8 * g + 8):
            out.append(_dot(h, jnp.concatenate([a_weight(m, hh) for m in range(3)], axis=1)))
        return out

    def a_scores(heads):
        out = []
        for p in range(0, 8, 2):
            y = jnp.concatenate(heads[p:p + 2], axis=0)
            q = y[:, 0:128].astype(BF16)
            k = jnp.concatenate([y[:, 128:256], pad], axis=0).astype(BF16)
            s = lax.dot_general(q, k, (((1,), (1,)), ((), ())), preferred_element_type=F32)
            out.append((s, y[:, 256:384]))
        return out

    def a_values(scored):
        out = []
        for s, v in scored:
            s = s * gain + bias
            top = jnp.max(s, axis=-1, keepdims=True)
            e = jnp.exp2(s - top)
            v = jnp.concatenate([v, pad], axis=0).astype(BF16)
            o = _dot(e.astype(BF16), v) * _reciprocal(jnp.sum(e, axis=-1, keepdims=True))
            out += [o[:L], o[L:]]
        return out

    def a_output(o, g):
        lhs = jnp.concatenate(o, axis=1).astype(BF16)
        w = jnp.concatenate(
            [_bf16_rows(wo_words[n, g * 512:(g + 1) * 512, :]) for n in range(8)], axis=1)
        return _dot(lhs, w)

    def a_segment(h, pick_rows, out_rows, filler):
        y, s, o, acc = [None] * 4, [None] * 4, [None] * 4, None

        def attend(g):
            s[g] = a_scores([pick_rows(8 * g + k, y[g][k]) for k in range(8)])

        def emit(g):
            part = a_output([out_rows(8 * g + k, o[g][k]) for k in range(8)], g)
            if g == 0:
                accum[0:part.shape[0], :] = part
            elif g < 3:
                accum[0:part.shape[0], :] += part
            else:
                return accum[0:part.shape[0], :] + part

        y[0] = a_project(h, 0)
        y[1] = a_project(h, 1)
        attend(0)
        y[2] = a_project(h, 2)
        o[0] = a_values(s[0])
        attend(1)
        y[3] = a_project(h, 3)
        o[1] = a_values(s[1])
        attend(2)
        acc = emit(0)
        attend(3)
        o[2] = a_values(s[2])
        acc = emit(1)
        o[3] = a_values(s[3])
        acc = emit(2)
        acc = emit(3)
        filler()
        return sum(y, []), sum(o, []), acc

    def b_attention(t0):
        base = pl.ds(pl.multiple_of(t0, SEG), HALO + SEG)
        lane = lax.broadcasted_iota(jnp.int32, (SEG, 128), 1)
        pos = lax.broadcasted_iota(jnp.int32, (SEG, 128), 0) + t0

        def window(j, w):
            return qkvb.at[j, base][HALO - w * DIL:HALO - w * DIL + SEG, :]

        def exchange_sum(x, v):
            return x + jnp.where((lane & v) == 0, pltpu.roll(x, 128 - v, 1), pltpu.roll(x, v, 1))

        q = [window(j, 0) for j in range(8)]
        logits = []
        for w in range(WIN):
            acc = q[0] * window(8, w)
            for j in range(1, 8):
                acc = acc + q[j] * window(8 + j, w)
            acc = exchange_sum(exchange_sum(acc, 16), 1) * (DHB ** -0.5 * LOG2E)
            logits.append(jnp.where(pos >= w * DIL, acc, NEG * LOG2E) if w else acc)
        top = logits[0]
        for x in logits[1:]:
            top = jnp.maximum(top, x)
        e = [jnp.exp2(x - top) for x in logits]
        total = e[0]
        for x in e[1:]:
            total = total + x
        inv = _reciprocal(total)
        p = [x * inv for x in e]
        out = []
        for j in range(8):
            acc = p[0] * window(16 + j, 0)
            for w in range(1, WIN):
                acc = acc + p[w] * window(16 + j, w)
            out.append(acc)
        return jnp.concatenate(out, axis=1).astype(BF16)

    def two_segments(mem, t0, out):
        def b_block(k):
            def run():
                o = b_attention(t0 + k * SEG)
                w = jnp.concatenate([
                    jnp.concatenate([wob[r * PITCH_B:r * PITCH_B + 64, :]
                                     for r in range(8 * n, 8 * n + 8)], axis=0)
                    for n in range(D // 128)], axis=1)
                out[k * SEG:(k + 1) * SEG, D:2 * D] = _dot(o, _bf16_rows(w)).astype(BF16)
            return run

        x = xa[pl.ds(pl.multiple_of(t0, 2 * SEG), 2 * SEG), :].astype(F32)

        h = jnp.concatenate([mem, x[:SEG + 8]], axis=0).astype(BF16)
        y0, o0, out0 = a_segment(
            h, lambda hh, y: y[:L], lambda hh, o: o[:L - 8], b_block(0))
        out[0:SEG - 8, 0:D] = out0[NMEM:].astype(BF16)

        h = jnp.concatenate([out0[:NMEM], x[SEG + 8:]], axis=0).astype(BF16)
        _, _, out1 = a_segment(
            h,
            lambda hh, y: jnp.concatenate([y[:NMEM], y0[hh][L:], y[NMEM:]], axis=0),
            lambda hh, o: jnp.concatenate([o[:NMEM], o0[hh][L - 8:], o[NMEM:]], axis=0),
            b_block(1))
        out[SEG - 8:2 * SEG, 0:D] = out1[NMEM:].astype(BF16)
        return out1[:NMEM]

    def step(i, mem):
        slot = i % 2

        @pl.when(i >= 2)
        def _():
            out_copy(i - 2, slot).wait()

        @pl.when(i == XA_HEAD // ROWS)
        def _():
            wait_next_batch()

        for r in range(0, ROWS, 2 * SEG):
            mem = two_segments(mem, i * ROWS + r, ostage.at[slot, r:r + 2 * SEG])
        out_copy(i, slot).start()
        return mem

    steps = S // ROWS
    lax.fori_loop(0, steps, step, mem0_ref[...].astype(F32))
    for i in (steps - 2, steps - 1):
        out_copy(i, i % 2).wait()


def pallas_concat_heads__memory_aug_recurrent_mem_tr__sliding_local_dilated__prompt_kernel(
    A_x, A_mem0, A_Wq, A_Wk, A_Wv, A_Wo, A_seg_len, B_x, B_wqkv, B_wo,
):
    assert A_seg_len == SEG and A_x.shape == (1, S, D) and A_mem0.shape == (1, NMEM, D)
    assert A_Wq.shape == (D, HA, DHA) and B_x.shape == (1, S, D)
    hbm = pl.BlockSpec(memory_space=pl.ANY)
    chunked = (D // 16, 16 * HA, DHA)
    out = pl.pallas_call(
        _kernel,
        out_shape=jax.ShapeDtypeStruct((S, 2 * D), BF16),
        in_specs=[pl.BlockSpec(memory_space=pltpu.SMEM), hbm,
                  pl.BlockSpec(memory_space=pltpu.VMEM)] + [hbm] * 7,
        out_specs=hbm,
        scratch_shapes=[
            pltpu.VMEM((3 * HA * PITCH_A, 128), U32),
            pltpu.VMEM((8, HA * DHA, 128), BF16),
            pltpu.VMEM((3, D // 2, D), U32),
            pltpu.VMEM((64 * PITCH_B, 128), U32),
            pltpu.VMEM((3,) + chunked, BF16),
            pltpu.VMEM((D, 3 * D), BF16),
            pltpu.VMEM((8, D, 128), BF16),
            pltpu.VMEM((24, HALO + S, 128), F32),
            pltpu.VMEM((S, D), BF16),
            pltpu.VMEM((S, D), BF16),
            pltpu.VMEM((2, ROWS, 2 * D), BF16),
            pltpu.VMEM((48, D), F32),
            pltpu.SemaphoreType.DMA((D // KC + 8,)),
            pltpu.SemaphoreType.DMA((2,)),
        ],
        compiler_params=pltpu.CompilerParams(vmem_limit_bytes=120 * 1024 * 1024),
    )(
        np.zeros((1,), np.int32),
        A_x.reshape(S, D), A_mem0.reshape(NMEM, D),
        A_Wq.reshape(chunked), A_Wk.reshape(chunked), A_Wv.reshape(chunked),
        A_Wo.reshape(HA * DHA, D),
        B_x.reshape(S, D), B_wqkv, B_wo,
    )
    return out.reshape(1, S, 2 * D)
```

```python
import functools

import numpy as np
import jax
import jax.numpy as jnp
from jax import lax
import jax.experimental.pallas as pl
import jax.experimental.pallas.tpu as pltpu

F32, BF16, U32 = jnp.float32, jnp.bfloat16, jnp.uint32

S = 2048
D = 1024
HA, DHA = 32, 128
NMEM, SEG = 8, 32
HB, DHB = 32, 32
WIN, DIL = 8, 2
HALO = 16
NEG = -1000000000.0
LOG2E = float(np.log2(np.e))

RB = 512
RP = 128
ROWS = 2 * SEG
XA_HEAD = 256
K_SPLIT = (0, 128, 256, 512, 768, 1024)
A_SPLIT = (0, 24, 56, 64)
PITCH_A = D // 2 + 1
PITCH_B = 64 + 1


def _bf16_rows(words):
    return pltpu.bitcast(words, BF16)


def _dot(a, b):
    return jnp.dot(a, b, preferred_element_type=F32)


def _reciprocal(x):
    r = pl.reciprocal(x, approx=True)
    return r * (2.0 - x * r)


def _kernel(xa_hbm, mem0_ref, wq_hbm, wk_hbm, wv_hbm, wo_hbm, xb_hbm, wqkvb_hbm, wob_hbm,
            out_hbm,
            wa, wo, wb, wob, rawa0, rawa1, rawa2, rawb, rawob, qkvb, xa, xb, ostage, accum,
            sem_in, sem_out):

    def part(src, dst, *idx):
        return src.at[idx], dst.at[idx]

    rawa = (rawa0, rawa1, rawa2)

    def a_weights(n):
        return [(w.at[A_SPLIT[n]:A_SPLIT[n + 1]], rawa[n].at[m])
                for m, w in enumerate((wq_hbm, wk_hbm, wv_hbm))]

    def panels(src, dst):
        return [(src.at[:, n * 128:(n + 1) * 128], dst.at[n]) for n in range(D // 128)]

    every = slice(None)
    k_slices = [slice(lo, hi) for lo, hi in zip(K_SPLIT, K_SPLIT[1:])]
    wq_b = [part(wqkvb_hbm, rawb, ks, slice(0, D)) for ks in k_slices]
    x_b = [part(xb_hbm, xb, slice(0, RB), ks) for ks in k_slices]
    batches = [wq_b[:1]] + [list(pair) for pair in zip(wq_b[1:], x_b)] + [
        x_b[-1:],
        [part(xb_hbm, xb, slice(RB, 3 * RB))],
        [part(xb_hbm, xb, slice(3 * RB, S)), part(wqkvb_hbm, rawb, every, slice(D, 3 * D))],
        a_weights(0),
        a_weights(1),
        a_weights(2) + panels(wob_hbm, rawob),
        panels(wo_hbm, wo) + [part(xa_hbm, xa, slice(0, XA_HEAD))],
        [part(xa_hbm, xa, slice(XA_HEAD, S))],
    ]
    batches = [[pltpu.make_async_copy(src, dst, sem_in.at[n]) for src, dst in batch]
               for n, batch in enumerate(batches)]
    pending = iter(batches)

    def wait_next_batch():
        for copy in next(pending):
            copy.wait()

    def out_copy(i, slot):
        rows = pl.ds(pl.multiple_of(i * ROWS, ROWS), ROWS)
        return pltpu.make_async_copy(ostage.at[slot], out_hbm.at[rows], sem_out.at[slot])

    def permute_b_cols(chunk, row0, nrows):
        words = pltpu.bitcast(rawb[2 * row0:2 * (row0 + nrows), chunk * D:(chunk + 1) * D], U32)
        t = [words[:, g * 128:(g + 1) * 128] for g in range(8)]
        lane = lax.broadcasted_iota(jnp.int32, (nrows, 128), 1)
        for bit in (1, 2, 4):
            low = (lane & (2 * bit)) == 0
            for g in range(8):
                if not g & bit:
                    x, y = t[g], t[g | bit]
                    t[g] = jnp.where(low, x, pltpu.roll(y, 2 * bit, 1))
                    t[g | bit] = jnp.where(low, pltpu.roll(x, 128 - 2 * bit, 1), y)
        for g in range(8):
            wb[chunk, row0:row0 + nrows, g * 128:(g + 1) * 128] = t[g]

    def permute_b_out_rows(n, half, zeros):
        src = rawob.bitcast(U32)
        for a in range(32 * half, 32 * half + 32):
            start = n * 8 * PITCH_B + (a & 7) * 8 + (a >> 3)
            wob[pl.ds(start, 8, stride=PITCH_B), :] = src[n, a * 8:(a + 1) * 8, :] | zeros

    def repack_a(n, t, m, zeros):
        src = rawa[n].bitcast(U32)
        half_word = zeros | 16
        for i in range(8):
            for half in range(2):
                r = 32 * i + 8 * half
                even, odd = src[m, t, r:r + 8, :], src[m, t, r + 16:r + 24, :]
                start = (m * HA + 8 * half) * PITCH_A + 8 * (A_SPLIT[n] + t) + i
                wa[pl.ds(start, 8, stride=PITCH_A), :] = (
                    (even & np.uint32(0xFFFF)) | (odd << half_word))
                wa[pl.ds(start + HA // 2 * PITCH_A, 8, stride=PITCH_A), :] = (
                    (even >> half_word) | (odd & np.uint32(0xFFFF0000)))

    def repack_jobs(n, lo, hi):
        return [functools.partial(repack_a, n, t, m) for t in range(lo, hi) for m in range(3)]

    def a_weight(m, head):
        start = (m * HA + (head % 2) * (HA // 2) + head // 2) * PITCH_A
        return _bf16_rows(wa[start:start + D // 2, :])

    def project_b(chunk, r, side_jobs=()):
        y = _dot(xb[r * RP:(r + 1) * RP, :], _bf16_rows(wb[chunk]))
        for j in range(8):
            qkvb[chunk * 8 + j, HALO + r * RP:HALO + (r + 1) * RP, :] = y[:, j * 128:(j + 1) * 128]
        for k, job in enumerate(side_jobs):
            j, i = divmod(k * RP // len(side_jobs), RP // 8)
            done = y[8 * i:8 * i + 8, j * 128:(j + 1) * 128]
            job((pltpu.bitcast(done, U32) >> 16) >> 16)

    for batch in batches:
        for copy in batch:
            copy.start()

    wait_next_batch()
    permute_b_cols(0, 0, K_SPLIT[1] // 2)
    for c, ks in enumerate(k_slices):
        wait_next_batch()
        for r in range(RB // RP):
            rows = slice(HALO + r * RP, HALO + (r + 1) * RP)
            y = _dot(xb[r * RP:(r + 1) * RP, ks], _bf16_rows(wb[0, ks.start // 2:ks.stop // 2, :]))
            for j in range(8):
                piece = y[:, j * 128:(j + 1) * 128]
                qkvb[j, rows, :] = piece + qkvb[j, rows, :] if c else piece
        if c + 1 < len(k_slices):
            permute_b_cols(0, ks.stop // 2, (K_SPLIT[c + 2] - ks.stop) // 2)

    wait_next_batch()
    for r in range(4, 12):
        project_b(0, r)
    wait_next_batch()
    for r in range(4):
        project_b(0, 12 + r)
        permute_b_cols(1, r * D // 8, D // 8)
    for r in range(4):
        project_b(1, r)
        permute_b_cols(2, r * D // 8, D // 8)
    wait_next_batch()
    for r in range(12):
        project_b(1, 4 + r, repack_jobs(0, 2 * r, 2 * r + 2))
    wait_next_batch()
    for r in range(8):
        project_b(2, r, repack_jobs(1, 4 * r, 4 * r + 4))
    wait_next_batch()
    for r in range(8):
        project_b(2, 8 + r, repack_jobs(2, r, r + 1)
                  + [functools.partial(permute_b_out_rows, r, half) for half in range(2)])

    for j in range(8, 24):
        qkvb[j, 0:HALO, :] = jnp.broadcast_to(qkvb[j, HALO:HALO + 1, :], (HALO, 128))
    wait_next_batch()

    L = NMEM + SEG
    row = lax.broadcasted_iota(jnp.int32, (2 * L, 128), 0)
    col = lax.broadcasted_iota(jnp.int32, (2 * L, 128), 1)
    same_head = ((row < L) == (col < L)) & (col < 2 * L)
    row = jnp.where(row < L, row, row - L)
    col = jnp.where(col < L, col, col - L)
    visible = same_head & ((row < NMEM) | (row >= col))
    gain = jnp.where(visible, DHA ** -0.5 * LOG2E, 0.0).astype(F32)
    bias = jnp.where(visible, 0.0, jnp.where(same_head, NEG * LOG2E, -jnp.inf)).astype(F32)
    wo_words = wo.bitcast(U32)
    pad = jnp.zeros((128 - 2 * L, 128), F32)

    def a_project(h, g):
        out = []
        for hh in range(8 * g, 8 * g + 8):
            out.append(_dot(h, jnp.concatenate([a_weight(m, hh) for m in range(3)], axis=1)))
        return out

    def a_scores(heads):
        out = []
        for p in range(0, 8, 2):
            y = jnp.concatenate(heads[p:p + 2], axis=0)
            q = y[:, 0:128].astype(BF16)
            k = jnp.concatenate([y[:, 128:256], pad], axis=0).astype(BF16)
            s = lax.dot_general(q, k, (((1,), (1,)), ((), ())), preferred_element_type=F32)
            out.append((s, y[:, 256:384]))
        return out

    def a_values(scored):
        out = []
        for s, v in scored:
            s = s * gain + bias
            top = jnp.max(s, axis=-1, keepdims=True)
            e = jnp.exp2(s - top)
            v = jnp.concatenate([v, pad], axis=0).astype(BF16)
            o = _dot(e.astype(BF16), v) * _reciprocal(jnp.sum(e, axis=-1, keepdims=True))
            out += [o[:L], o[L:]]
        return out

    def a_output(o, g):
        lhs = jnp.concatenate(o, axis=1).astype(BF16)
        w = jnp.concatenate(
            [_bf16_rows(wo_words[n, g * 512:(g + 1) * 512, :]) for n in range(8)], axis=1)
        return _dot(lhs, w)

    def a_segment(h, pick_rows, out_rows, filler):
        y, s, o, acc = [None] * 4, [None] * 4, [None] * 4, None

        def attend(g):
            s[g] = a_scores([pick_rows(8 * g + k, y[g][k]) for k in range(8)])

        def emit(g):
            part = a_output([out_rows(8 * g + k, o[g][k]) for k in range(8)], g)
            if g == 0:
                accum[0:part.shape[0], :] = part
            elif g < 3:
                accum[0:part.shape[0], :] += part
            else:
                return accum[0:part.shape[0], :] + part

        y[0] = a_project(h, 0)
        y[1] = a_project(h, 1)
        attend(0)
        y[2] = a_project(h, 2)
        o[0] = a_values(s[0])
        attend(1)
        y[3] = a_project(h, 3)
        o[1] = a_values(s[1])
        attend(2)
        acc = emit(0)
        attend(3)
        o[2] = a_values(s[2])
        acc = emit(1)
        o[3] = a_values(s[3])
        acc = emit(2)
        acc = emit(3)
        filler()
        return sum(y, []), sum(o, []), acc

    def b_attention(t0):
        base = pl.ds(pl.multiple_of(t0, SEG), HALO + SEG)
        lane = lax.broadcasted_iota(jnp.int32, (SEG, 128), 1)
        pos = lax.broadcasted_iota(jnp.int32, (SEG, 128), 0) + t0

        def window(j, w):
            return qkvb.at[j, base][HALO - w * DIL:HALO - w * DIL + SEG, :]

        def exchange_sum(x, v):
            return x + jnp.where((lane & v) == 0, pltpu.roll(x, 128 - v, 1), pltpu.roll(x, v, 1))

        q = [window(j, 0) for j in range(8)]
        logits = []
        for w in range(WIN):
            acc = q[0] * window(8, w)
            for j in range(1, 8):
                acc = acc + q[j] * window(8 + j, w)
            acc = exchange_sum(exchange_sum(acc, 16), 1) * (DHB ** -0.5 * LOG2E)
            logits.append(jnp.where(pos >= w * DIL, acc, NEG * LOG2E) if w else acc)
        top = logits[0]
        for x in logits[1:]:
            top = jnp.maximum(top, x)
        e = [jnp.exp2(x - top) for x in logits]
        total = e[0]
        for x in e[1:]:
            total = total + x
        inv = _reciprocal(total)
        p = [x * inv for x in e]
        out = []
        for j in range(8):
            acc = p[0] * window(16 + j, 0)
            for w in range(1, WIN):
                acc = acc + p[w] * window(16 + j, w)
            out.append(acc)
        return jnp.concatenate(out, axis=1).astype(BF16)

    def two_segments(mem, t0, out):
        def b_block(k):
            def run():
                o = b_attention(t0 + k * SEG)
                w = jnp.concatenate([
                    jnp.concatenate([wob[r * PITCH_B:r * PITCH_B + 64, :]
                                     for r in range(8 * n, 8 * n + 8)], axis=0)
                    for n in range(D // 128)], axis=1)
                out[k * SEG:(k + 1) * SEG, D:2 * D] = _dot(o, _bf16_rows(w)).astype(BF16)
            return run

        x = xa[pl.ds(pl.multiple_of(t0, 2 * SEG), 2 * SEG), :].astype(F32)

        h = jnp.concatenate([mem, x[:SEG + 8]], axis=0).astype(BF16)
        y0, o0, out0 = a_segment(
            h, lambda hh, y: y[:L], lambda hh, o: o[:L - 8], b_block(0))
        out[0:SEG - 8, 0:D] = out0[NMEM:].astype(BF16)

        h = jnp.concatenate([out0[:NMEM], x[SEG + 8:]], axis=0).astype(BF16)
        _, _, out1 = a_segment(
            h,
            lambda hh, y: jnp.concatenate([y[:NMEM], y0[hh][L:], y[NMEM:]], axis=0),
            lambda hh, o: jnp.concatenate([o[:NMEM], o0[hh][L - 8:], o[NMEM:]], axis=0),
            b_block(1))
        out[SEG - 8:2 * SEG, 0:D] = out1[NMEM:].astype(BF16)
        return out1[:NMEM]

    def step(i, mem):
        slot = i % 2

        @pl.when(i >= 2)
        def _():
            out_copy(i - 2, slot).wait()

        @pl.when(i == XA_HEAD // ROWS)
        def _():
            wait_next_batch()

        for r in range(0, ROWS, 2 * SEG):
            mem = two_segments(mem, i * ROWS + r, ostage.at[slot, r:r + 2 * SEG])
        out_copy(i, slot).start()
        return mem

    steps = S // ROWS
    lax.fori_loop(0, steps, step, mem0_ref[...].astype(F32))
    for i in (steps - 2, steps - 1):
        out_copy(i, i % 2).wait()


def pallas_concat_heads__memory_aug_recurrent_mem_tr__sliding_local_dilated__prompt_kernel(
    A_x, A_mem0, A_Wq, A_Wk, A_Wv, A_Wo, A_seg_len, B_x, B_wqkv, B_wo,
):
    assert A_seg_len == SEG and A_x.shape == (1, S, D) and A_mem0.shape == (1, NMEM, D)
    assert A_Wq.shape == (D, HA, DHA) and B_x.shape == (1, S, D)
    hbm = pl.BlockSpec(memory_space=pl.ANY)

    def padded_rows(n):
        return -(-n // 64) * 64

    chunked = (D // 16, 16 * HA, DHA)
    out = pl.pallas_call(
        _kernel,
        out_shape=jax.ShapeDtypeStruct((S, 2 * D), BF16),
        in_specs=[hbm, pl.BlockSpec(memory_space=pltpu.VMEM)] + [hbm] * 7,
        out_specs=hbm,
        scratch_shapes=[
            pltpu.VMEM((padded_rows((3 * HA + 1) * PITCH_A), 128), U32),
            pltpu.VMEM((8, HA * DHA, 128), BF16),
            pltpu.VMEM((3, D // 2, D), U32),
            pltpu.VMEM((padded_rows(65 * PITCH_B), 128), U32),
            *[pltpu.VMEM((3, hi - lo) + chunked[1:], BF16)
              for lo, hi in zip(A_SPLIT, A_SPLIT[1:])],
            pltpu.VMEM((D, 3 * D), BF16),
            pltpu.VMEM((8, D, 128), BF16),
            pltpu.VMEM((24, HALO + S, 128), F32),
            pltpu.VMEM((S, D), BF16),
            pltpu.VMEM((S, D), BF16),
            pltpu.VMEM((2, ROWS, 2 * D), BF16),
            pltpu.VMEM((48, D), F32),
            pltpu.SemaphoreType.DMA((len(K_SPLIT) + 6,)),
            pltpu.SemaphoreType.DMA((2,)),
        ],
        compiler_params=pltpu.CompilerParams(vmem_limit_bytes=120 * 1024 * 1024),
    )(
        A_x.reshape(S, D), A_mem0.reshape(NMEM, D),
        A_Wq.reshape(chunked), A_Wk.reshape(chunked), A_Wv.reshape(chunked),
        A_Wo.reshape(HA * DHA, D),
        B_x.reshape(S, D), B_wqkv, B_wo,
    )
    return out.reshape(1, S, 2 * D)
```

```python
import functools

import numpy as np
import jax
import jax.numpy as jnp
from jax import lax
import jax.experimental.pallas as pl
import jax.experimental.pallas.tpu as pltpu

F32, BF16, U32 = jnp.float32, jnp.bfloat16, jnp.uint32

S, D = 2048, 1024
HA, DHA = 32, 128
NMEM, SEG = 8, 32
DHB = 32
WIN, DIL = 8, 2
NEG = -1000000000.0
LOG2E = float(np.log2(np.e))

NT = D // 128
HALO = 16
RP = 128
FIRST = 1024
K_SPLIT = (0, 128, 256, 384, 512, D)
A_SPLIT = (0, 24, 56, D // 16)
XA_HEAD = 256
STEP = 2 * SEG
PITCH_A = D // 2 + 1
PITCH_B = 64 + 1


def _bf16_rows(words):
    return pltpu.bitcast(words, BF16)


def _dot(a, b):
    return jnp.dot(a, b, preferred_element_type=F32)


def _reciprocal(x):
    r = pl.reciprocal(x, approx=True)
    return r * (2.0 - x * r)


def _kernel(xa_hbm, mem0_ref, wq_hbm, wk_hbm, wv_hbm, wo_hbm, xb_hbm, wqkvb_hbm, wob_hbm,
            out_hbm,
            wa, wo, wb, wob, rawa0, rawa1, rawa2, rawb, rawob, qkvb, xa, xb, ostage, accum,
            sem_in, sem_out):
    rawa = (rawa0, rawa1, rawa2)

    def part(src, dst, *idx):
        return src.at[idx], dst.at[idx]

    def a_weights(n):
        return [(w.at[A_SPLIT[n]:A_SPLIT[n + 1]], rawa[n].at[m])
                for m, w in enumerate((wq_hbm, wk_hbm, wv_hbm))]

    def panels(src, dst):
        return [(src.at[:, n * 128:(n + 1) * 128], dst.at[n]) for n in range(NT)]

    k_slices = [slice(lo, hi) for lo, hi in zip(K_SPLIT, K_SPLIT[1:])]
    wq_b = [part(wqkvb_hbm, rawb, ks, slice(0, D)) for ks in k_slices]
    x_b = [part(xb_hbm, xb, slice(0, FIRST), ks) for ks in k_slices]
    batches = [wq_b[:1]] + [list(pair) for pair in zip(wq_b[1:], x_b)] + [
        x_b[-1:],
        [part(xb_hbm, xb, slice(FIRST, S))],
        [part(wqkvb_hbm, rawb, slice(0, D), slice(D, 3 * D))],
        a_weights(0),
        a_weights(1),
        a_weights(2) + panels(wob_hbm, rawob),
        panels(wo_hbm, wo) + [part(xa_hbm, xa, slice(0, XA_HEAD))],
        [part(xa_hbm, xa, slice(XA_HEAD, S))],
    ]
    assert len(batches) == sem_in.shape[0]
    batches = [[pltpu.make_async_copy(src, dst, sem_in.at[n]) for src, dst in batch]
               for n, batch in enumerate(batches)]
    pending = iter(batches)

    def wait_next_batch():
        for copy in next(pending):
            copy.wait()

    def out_copy(i, slot):
        rows = pl.ds(pl.multiple_of(i * STEP, STEP), STEP)
        return pltpu.make_async_copy(ostage.at[slot], out_hbm.at[rows], sem_out.at[slot])

    def permute_b_cols(chunk, row0, nrows):
        words = pltpu.bitcast(rawb[2 * row0:2 * (row0 + nrows), chunk * D:(chunk + 1) * D], U32)
        t = [words[:, g * 128:(g + 1) * 128] for g in range(NT)]
        lane = lax.broadcasted_iota(jnp.int32, (nrows, 128), 1)
        for bit in (1, 2, 4):
            low = (lane & (2 * bit)) == 0
            for g in range(NT):
                if not g & bit:
                    x, y = t[g], t[g | bit]
                    t[g] = jnp.where(low, x, pltpu.roll(y, 2 * bit, 1))
                    t[g | bit] = jnp.where(low, pltpu.roll(x, 128 - 2 * bit, 1), y)
        for g in range(NT):
            wb[chunk, row0:row0 + nrows, g * 128:(g + 1) * 128] = t[g]

    def permute_b_out_rows(n, half, zeros):
        src = rawob.bitcast(U32)
        for a in range(32 * half, 32 * half + 32):
            start = n * 8 * PITCH_B + (a & 7) * 8 + (a >> 3)
            wob[pl.ds(start, 8, stride=PITCH_B), :] = src[n, a * 8:(a + 1) * 8, :] | zeros

    def b_out_weight():
        return _bf16_rows(jnp.concatenate([
            jnp.concatenate([wob[r * PITCH_B:r * PITCH_B + 64, :]
                             for r in range(8 * n, 8 * n + 8)], axis=0)
            for n in range(NT)], axis=1))

    def repack_a(n, t, m, zeros):
        src = rawa[n].bitcast(U32)
        half_word = zeros | 16
        for i in range(8):
            for half in range(2):
                r = 32 * i + 8 * half
                even, odd = src[m, t, r:r + 8, :], src[m, t, r + 16:r + 24, :]
                start = (m * HA + 8 * half) * PITCH_A + 8 * (A_SPLIT[n] + t) + i
                wa[pl.ds(start, 8, stride=PITCH_A), :] = (
                    (even & np.uint32(0xFFFF)) | (odd << half_word))
                wa[pl.ds(start + HA // 2 * PITCH_A, 8, stride=PITCH_A), :] = (
                    (even >> half_word) | (odd & np.uint32(0xFFFF0000)))

    def repack_jobs(n, lo, hi):
        return [functools.partial(repack_a, n, t, m) for t in range(lo, hi) for m in range(3)]

    def a_weight(m, head):
        start = (m * HA + (head % 2) * (HA // 2) + head // 2) * PITCH_A
        return _bf16_rows(wa[start:start + D // 2, :])

    def project_b(chunk, r, side_jobs=()):
        y = _dot(xb[r * RP:(r + 1) * RP, :], _bf16_rows(wb[chunk]))
        for j in range(NT):
            qkvb[chunk * NT + j, HALO + r * RP:HALO + (r + 1) * RP, :] = y[:, j * 128:(j + 1) * 128]
        for k, job in enumerate(side_jobs):
            j, i = divmod(k * RP // len(side_jobs), RP // 8)
            done = y[8 * i:8 * i + 8, j * 128:(j + 1) * 128]
            job((pltpu.bitcast(done, U32) >> 16) >> 16)

    for batch in batches:
        for copy in batch:
            copy.start()

    wait_next_batch()
    permute_b_cols(0, 0, K_SPLIT[1] // 2)
    for c, ks in enumerate(k_slices):
        wait_next_batch()
        for r in range(FIRST // RP):
            rows = slice(HALO + r * RP, HALO + (r + 1) * RP)
            y = _dot(xb[r * RP:(r + 1) * RP, ks], _bf16_rows(wb[0, ks.start // 2:ks.stop // 2, :]))
            for j in range(NT):
                piece = y[:, j * 128:(j + 1) * 128]
                qkvb[j, rows, :] = piece + qkvb[j, rows, :] if c else piece
        if c + 1 < len(k_slices):
            permute_b_cols(0, ks.stop // 2, (K_SPLIT[c + 2] - ks.stop) // 2)

    wait_next_batch()
    for r in range(FIRST // RP, 12):
        project_b(0, r)
    wait_next_batch()
    for r in range(4):
        project_b(0, 12 + r)
        permute_b_cols(1, r * D // 8, D // 8)
    for r in range(4):
        project_b(1, r)
        permute_b_cols(2, r * D // 8, D // 8)
    wait_next_batch()
    for r in range(12):
        project_b(1, 4 + r, repack_jobs(0, 2 * r, 2 * r + 2))
    wait_next_batch()
    for r in range(8):
        project_b(2, r, repack_jobs(1, 4 * r, 4 * r + 4))
    wait_next_batch()
    for r in range(8):
        project_b(2, 8 + r, repack_jobs(2, r, r + 1)
                  + [functools.partial(permute_b_out_rows, r, half) for half in range(2)])

    for j in range(NT, 3 * NT):
        qkvb[j, 0:HALO, :] = jnp.broadcast_to(qkvb[j, HALO:HALO + 1, :], (HALO, 128))
    wait_next_batch()

    L = NMEM + SEG
    row = lax.broadcasted_iota(jnp.int32, (2 * L, 128), 0)
    col = lax.broadcasted_iota(jnp.int32, (2 * L, 128), 1)
    same_head = ((row < L) == (col < L)) & (col < 2 * L)
    row = jnp.where(row < L, row, row - L)
    col = jnp.where(col < L, col, col - L)
    visible = same_head & ((row < NMEM) | (row >= col))
    gain = jnp.where(visible, DHA ** -0.5 * LOG2E, 0.0).astype(F32)
    bias = jnp.where(visible, 0.0, jnp.where(same_head, NEG * LOG2E, -jnp.inf)).astype(F32)
    pad = jnp.zeros((128 - 2 * L, 128), F32)
    wo_words = wo.bitcast(U32)

    def a_project(h, g):
        return [_dot(h, jnp.concatenate([a_weight(m, head) for m in range(3)], axis=1))
                for head in range(8 * g, 8 * g + 8)]

    def a_scores(heads):
        out = []
        for p in range(0, 8, 2):
            y = jnp.concatenate(heads[p:p + 2], axis=0)
            q = y[:, 0:128].astype(BF16)
            k = jnp.concatenate([y[:, 128:256], pad], axis=0).astype(BF16)
            s = lax.dot_general(q, k, (((1,), (1,)), ((), ())), preferred_element_type=F32)
            out.append((s, y[:, 256:384]))
        return out

    def a_values(scored):
        out = []
        for s, v in scored:
            s = s * gain + bias
            e = jnp.exp2(s - jnp.max(s, axis=-1, keepdims=True))
            v = jnp.concatenate([v, pad], axis=0).astype(BF16)
            o = _dot(e.astype(BF16), v) * _reciprocal(jnp.sum(e, axis=-1, keepdims=True))
            out += [o[:L], o[L:]]
        return out

    def a_output(o, g):
        w = jnp.concatenate(
            [_bf16_rows(wo_words[n, g * 512:(g + 1) * 512, :]) for n in range(NT)], axis=1)
        return _dot(jnp.concatenate(o, axis=1).astype(BF16), w)

    def a_segment(h, attend_rows, output_rows, filler):
        y, s, o = [None] * 4, [None] * 4, [None] * 4

        def attend(g):
            s[g] = a_scores([attend_rows(8 * g + k, y[g][k]) for k in range(8)])

        def emit(g):
            return a_output([output_rows(8 * g + k, o[g][k]) for k in range(8)], g)

        y[0] = a_project(h, 0)
        y[1] = a_project(h, 1)
        attend(0)
        y[2] = a_project(h, 2)
        o[0] = a_values(s[0])
        attend(1)
        y[3] = a_project(h, 3)
        o[1] = a_values(s[1])
        attend(2)
        first = emit(0)
        rows = slice(0, first.shape[0])
        accum[rows, :] = first
        o[2] = a_values(s[2])
        attend(3)
        accum[rows, :] += emit(1)
        o[3] = a_values(s[3])
        accum[rows, :] += emit(2)
        last = emit(3)
        out = accum[rows, :] + last
        filler()
        return sum(y, []), sum(o, []), out

    def b_attention(t0):
        base = pl.ds(pl.multiple_of(t0, SEG), HALO + SEG)
        lane = lax.broadcasted_iota(jnp.int32, (SEG, 128), 1)
        pos = lax.broadcasted_iota(jnp.int32, (SEG, 128), 0) + t0

        def window(j, w):
            return qkvb.at[j, base][HALO - w * DIL:HALO - w * DIL + SEG, :]

        def exchange_sum(x, v):
            return x + jnp.where((lane & v) == 0, pltpu.roll(x, 128 - v, 1), pltpu.roll(x, v, 1))

        q = [window(j, 0) for j in range(NT)]
        logits = []
        for w in range(WIN):
            acc = q[0] * window(NT, w)
            for j in range(1, NT):
                acc = acc + q[j] * window(NT + j, w)
            acc = exchange_sum(exchange_sum(acc, 16), 1) * (DHB ** -0.5 * LOG2E)
            logits.append(jnp.where(pos >= w * DIL, acc, NEG * LOG2E) if w else acc)
        top = functools.reduce(jnp.maximum, logits)
        e = [jnp.exp2(x - top) for x in logits]
        inv = _reciprocal(functools.reduce(jnp.add, e))
        p = [x * inv for x in e]
        out = []
        for j in range(NT):
            acc = p[0] * window(2 * NT + j, 0)
            for w in range(1, WIN):
                acc = acc + p[w] * window(2 * NT + j, w)
            out.append(acc)
        return jnp.concatenate(out, axis=1).astype(BF16)

    def step(i, mem):
        slot = i % 2
        t0 = i * STEP

        @pl.when(i >= 2)
        def _():
            out_copy(i - 2, slot).wait()

        @pl.when(i == XA_HEAD // STEP)
        def _():
            wait_next_batch()

        def b_block(k):
            o = b_attention(t0 + k * SEG)
            ostage[slot, k * SEG:(k + 1) * SEG, D:2 * D] = _dot(o, b_out_weight()).astype(BF16)

        x = xa[pl.ds(pl.multiple_of(t0, STEP), STEP), :].astype(F32)

        h = jnp.concatenate([mem, x[:SEG + 8]], axis=0).astype(BF16)
        y0, o0, out0 = a_segment(
            h, lambda head, y: y[:L], lambda head, o: o[:L - 8], functools.partial(b_block, 0))
        ostage[slot, 0:SEG - 8, 0:D] = out0[NMEM:].astype(BF16)

        h = jnp.concatenate([out0[:NMEM], x[SEG + 8:]], axis=0).astype(BF16)
        _, _, out1 = a_segment(
            h,
            lambda head, y: jnp.concatenate([y[:NMEM], y0[head][L:], y[NMEM:]], axis=0),
            lambda head, o: jnp.concatenate([o[:NMEM], o0[head][L - 8:], o[NMEM:]], axis=0),
            functools.partial(b_block, 1))
        ostage[slot, SEG - 8:STEP, 0:D] = out1[NMEM:].astype(BF16)

        out_copy(i, slot).start()
        return out1[:NMEM]

    steps = S // STEP
    lax.fori_loop(0, steps, step, mem0_ref[...].astype(F32))
    for i in (steps - 2, steps - 1):
        out_copy(i, i % 2).wait()


def _word_rows(n):
    return pltpu.VMEM((-(-n // 64) * 64, 128), U32)


@functools.partial(jax.jit, static_argnames=("A_seg_len",))
def pallas_concat_heads__memory_aug_recurrent_mem_tr__sliding_local_dilated__prompt_kernel(
    A_x, A_mem0, A_Wq, A_Wk, A_Wv, A_Wo, A_seg_len, B_x, B_wqkv, B_wo,
):
    assert A_seg_len == SEG and A_x.shape == (1, S, D) and A_mem0.shape == (1, NMEM, D)
    assert A_Wq.shape == (D, HA, DHA) and B_x.shape == (1, S, D)
    hbm = pl.BlockSpec(memory_space=pl.ANY)
    grouped = (D // 16, 16 * HA, DHA)
    out = pl.pallas_call(
        _kernel,
        out_shape=jax.ShapeDtypeStruct((S, 2 * D), BF16),
        in_specs=[hbm, pl.BlockSpec(memory_space=pltpu.VMEM)] + [hbm] * 7,
        out_specs=hbm,
        scratch_shapes=[
            _word_rows((3 * HA + 1) * PITCH_A),
            pltpu.VMEM((NT, HA * DHA, 128), BF16),
            pltpu.VMEM((3, D // 2, D), U32),
            _word_rows((8 * NT + 1) * PITCH_B),
            *[pltpu.VMEM((3, hi - lo) + grouped[1:], BF16)
              for lo, hi in zip(A_SPLIT, A_SPLIT[1:])],
            pltpu.VMEM((D, 3 * D), BF16),
            pltpu.VMEM((NT, D, 128), BF16),
            pltpu.VMEM((3 * NT, HALO + S, 128), F32),
            pltpu.VMEM((S, D), BF16),
            pltpu.VMEM((S, D), BF16),
            pltpu.VMEM((2, STEP, 2 * D), BF16),
            pltpu.VMEM((NMEM + SEG + 8, D), F32),
            pltpu.SemaphoreType.DMA((len(K_SPLIT) + 7,)),
            pltpu.SemaphoreType.DMA((2,)),
        ],
        compiler_params=pltpu.CompilerParams(vmem_limit_bytes=120 * 1024 * 1024),
    )(
        A_x.reshape(S, D), A_mem0.reshape(NMEM, D),
        A_Wq.reshape(grouped), A_Wk.reshape(grouped), A_Wv.reshape(grouped),
        A_Wo.reshape(HA * DHA, D),
        B_x.reshape(S, D), B_wqkv, B_wo,
    )
    return out.reshape(1, S, 2 * D)
```

```python
import functools

import numpy as np
import jax
import jax.numpy as jnp
from jax import lax
import jax.experimental.pallas as pl
import jax.experimental.pallas.tpu as pltpu

F32, BF16, U32 = jnp.float32, jnp.bfloat16, jnp.uint32

S, D = 2048, 1024
HA, DHA = 32, 128
NMEM, SEG = 8, 32
DHB = 32
WIN, DIL = 8, 2
NEG = -1000000000.0
LOG2E = float(np.log2(np.e))

NT = D // 128
HALO = 16
RP = 128
FIRST = 1024
K_SPLIT = (0, 128, 256, 384, 512, D)
A_SPLIT = (0, 24, 56, D // 16)
XA_HEAD = 256
STEP = 2 * SEG
PITCH_A = D // 2 + 1
PITCH_B = 64 + 1


def _bf16_rows(words):
    return pltpu.bitcast(words, BF16)


def _dot(a, b):
    return jnp.dot(a, b, preferred_element_type=F32)


def _reciprocal(x):
    r = pl.reciprocal(x, approx=True)
    return r * (2.0 - x * r)


def _kernel(xa_hbm, mem0_ref, wq_hbm, wk_hbm, wv_hbm, wo_hbm, xb_hbm, wqkvb_hbm, wob_hbm,
            out_hbm,
            wa, wo, wb, wob, rawa0, rawa1, rawa2, rawb, rawob, qkvb, xa, xb, ostage, accum,
            sem_in, sem_out):
    rawa = (rawa0, rawa1, rawa2)

    def part(src, dst, *idx):
        return src.at[idx], dst.at[idx]

    def a_weights(n):
        return [(w.at[A_SPLIT[n]:A_SPLIT[n + 1]], rawa[n].at[m])
                for m, w in enumerate((wq_hbm, wk_hbm, wv_hbm))]

    def panels(src, dst):
        return [(src.at[:, n * 128:(n + 1) * 128], dst.at[n]) for n in range(NT)]

    k_slices = [slice(lo, hi) for lo, hi in zip(K_SPLIT, K_SPLIT[1:])]
    wq_b = [part(wqkvb_hbm, rawb, ks, slice(0, D)) for ks in k_slices]
    x_b = [part(xb_hbm, xb, slice(0, FIRST), ks) for ks in k_slices]
    batches = [wq_b[:1]] + [list(pair) for pair in zip(wq_b[1:], x_b)] + [
        x_b[-1:],
        [part(xb_hbm, xb, slice(FIRST, S))],
        [part(wqkvb_hbm, rawb, slice(0, D), slice(D, 3 * D))],
        a_weights(0),
        a_weights(1),
        a_weights(2) + panels(wob_hbm, rawob),
        panels(wo_hbm, wo) + [part(xa_hbm, xa, slice(0, XA_HEAD))],
        [part(xa_hbm, xa, slice(XA_HEAD, S))],
    ]
    assert len(batches) == sem_in.shape[0]
    batches = [[pltpu.make_async_copy(src, dst, sem_in.at[n]) for src, dst in batch]
               for n, batch in enumerate(batches)]
    pending = iter(batches)

    def wait_next_batch():
        for copy in next(pending):
            copy.wait()

    def out_copy(i, slot):
        rows = pl.ds(pl.multiple_of(i * STEP, STEP), STEP)
        return pltpu.make_async_copy(ostage.at[slot], out_hbm.at[rows], sem_out.at[slot])

    def permute_b_cols(chunk, row0, nrows):
        words = pltpu.bitcast(rawb[2 * row0:2 * (row0 + nrows), chunk * D:(chunk + 1) * D], U32)
        t = [words[:, g * 128:(g + 1) * 128] for g in range(NT)]
        lane = lax.broadcasted_iota(jnp.int32, (nrows, 128), 1)
        for bit in (1, 2, 4):
            low = (lane & (2 * bit)) == 0
            for g in range(NT):
                if not g & bit:
                    x, y = t[g], t[g | bit]
                    t[g] = jnp.where(low, x, pltpu.roll(y, 2 * bit, 1))
                    t[g | bit] = jnp.where(low, pltpu.roll(x, 128 - 2 * bit, 1), y)
        for g in range(NT):
            wb[chunk, row0:row0 + nrows, g * 128:(g + 1) * 128] = t[g]

    def permute_b_out_rows(n, half, zeros):
        words = rawob.bitcast(U32)[n, 256 * half:256 * (half + 1), :].reshape(32, 8, 128) | zeros
        for a in range(32 * half, 32 * half + 32):
            start = n * 8 * PITCH_B + (a & 7) * 8 + (a >> 3)
            wob[pl.ds(start, 8, stride=PITCH_B), :] = words[a % 32]

    def b_out_weight():
        return _bf16_rows(jnp.concatenate([
            jnp.concatenate([wob[r * PITCH_B:r * PITCH_B + 64, :]
                             for r in range(8 * n, 8 * n + 8)], axis=0)
            for n in range(NT)], axis=1))

    def repack_a(n, t, m, zeros):
        words = rawa[n].bitcast(U32)[m, t].reshape(8, 2, 2, 8, 128)
        even, odd = words[:, 0], words[:, 1]
        half_word = zeros | 16
        by_parity = ((even & np.uint32(0xFFFF)) | (odd << half_word),
                     (even >> half_word) | (odd & np.uint32(0xFFFF0000)))
        for i in range(8):
            for half in range(2):
                for parity in range(2):
                    panel = m * HA + parity * (HA // 2) + 8 * half
                    start = panel * PITCH_A + 8 * (A_SPLIT[n] + t) + i
                    wa[pl.ds(start, 8, stride=PITCH_A), :] = by_parity[parity][i, half]

    def repack_jobs(n, lo, hi):
        return [functools.partial(repack_a, n, t, m) for t in range(lo, hi) for m in range(3)]

    def a_weight(m, head):
        start = (m * HA + (head % 2) * (HA // 2) + head // 2) * PITCH_A
        return _bf16_rows(wa[start:start + D // 2, :])

    def project_b(chunk, r, side_jobs=()):
        y = _dot(xb[r * RP:(r + 1) * RP, :], _bf16_rows(wb[chunk]))
        for j in range(NT):
            qkvb[chunk * NT + j, HALO + r * RP:HALO + (r + 1) * RP, :] = y[:, j * 128:(j + 1) * 128]
        for k, job in enumerate(side_jobs):
            j, i = divmod(k * RP // len(side_jobs), RP // 8)
            done = y[8 * i:8 * i + 8, j * 128:(j + 1) * 128]
            job((pltpu.bitcast(done, U32) >> 16) >> 16)

    for batch in batches:
        for copy in batch:
            copy.start()

    wait_next_batch()
    permute_b_cols(0, 0, K_SPLIT[1] // 2)
    for c, ks in enumerate(k_slices):
        wait_next_batch()
        for r in range(FIRST // RP):
            rows = slice(HALO + r * RP, HALO + (r + 1) * RP)
            y = _dot(xb[r * RP:(r + 1) * RP, ks], _bf16_rows(wb[0, ks.start // 2:ks.stop // 2, :]))
            for j in range(NT):
                piece = y[:, j * 128:(j + 1) * 128]
                qkvb[j, rows, :] = piece + qkvb[j, rows, :] if c else piece
        if c + 1 < len(k_slices):
            permute_b_cols(0, ks.stop // 2, (K_SPLIT[c + 2] - ks.stop) // 2)

    wait_next_batch()
    for r in range(FIRST // RP, 12):
        project_b(0, r)
    wait_next_batch()
    for r in range(4):
        project_b(0, 12 + r)
        permute_b_cols(1, r * D // 8, D // 8)
    for r in range(4):
        project_b(1, r)
        permute_b_cols(2, r * D // 8, D // 8)
    wait_next_batch()
    for r in range(12):
        project_b(1, 4 + r, repack_jobs(0, 2 * r, 2 * r + 2))
    wait_next_batch()
    for r in range(8):
        project_b(2, r, repack_jobs(1, 4 * r, 4 * r + 4))
    wait_next_batch()
    for r in range(8):
        project_b(2, 8 + r, repack_jobs(2, r, r + 1)
                  + [functools.partial(permute_b_out_rows, r, half) for half in range(2)])

    for j in range(NT, 3 * NT):
        qkvb[j, 0:HALO, :] = jnp.broadcast_to(qkvb[j, HALO:HALO + 1, :], (HALO, 128))
    wait_next_batch()

    L = NMEM + SEG
    row = lax.broadcasted_iota(jnp.int32, (2 * L, 128), 0)
    col = lax.broadcasted_iota(jnp.int32, (2 * L, 128), 1)
    same_head = ((row < L) == (col < L)) & (col < 2 * L)
    row = jnp.where(row < L, row, row - L)
    col = jnp.where(col < L, col, col - L)
    visible = same_head & ((row < NMEM) | (row >= col))
    gain = jnp.where(visible, DHA ** -0.5 * LOG2E, 0.0).astype(F32)
    bias = jnp.where(visible, 0.0, jnp.where(same_head, NEG * LOG2E, -jnp.inf)).astype(F32)
    pad = jnp.zeros((128 - 2 * L, 128), F32)
    wo_words = wo.bitcast(U32)

    def a_project(h, g):
        return [_dot(h, jnp.concatenate([a_weight(m, head) for m in range(3)], axis=1))
                for head in range(8 * g, 8 * g + 8)]

    def a_scores(heads):
        out = []
        for p in range(0, 8, 2):
            y = jnp.concatenate(heads[p:p + 2], axis=0)
            q = y[:, 0:128].astype(BF16)
            k = jnp.concatenate([y[:, 128:256], pad], axis=0).astype(BF16)
            s = lax.dot_general(q, k, (((1,), (1,)), ((), ())), preferred_element_type=F32)
            out.append((s, y[:, 256:384]))
        return out

    def a_values(scored):
        out = []
        for s, v in scored:
            s = s * gain + bias
            e = jnp.exp2(s - jnp.max(s, axis=-1, keepdims=True))
            v = jnp.concatenate([v, pad], axis=0).astype(BF16)
            o = _dot(e.astype(BF16), v) * _reciprocal(jnp.sum(e, axis=-1, keepdims=True))
            out += [o[:L], o[L:]]
        return out

    def a_output(o, g):
        w = jnp.concatenate(
            [_bf16_rows(wo_words[n, g * 512:(g + 1) * 512, :]) for n in range(NT)], axis=1)
        return _dot(jnp.concatenate(o, axis=1).astype(BF16), w)

    def a_segment(h, attend_rows, output_rows, filler):
        y, s, o = [None] * 4, [None] * 4, [None] * 4

        def attend(g):
            s[g] = a_scores([attend_rows(8 * g + k, y[g][k]) for k in range(8)])

        def emit(g):
            return a_output([output_rows(8 * g + k, o[g][k]) for k in range(8)], g)

        y[0] = a_project(h, 0)
        y[1] = a_project(h, 1)
        attend(0)
        y[2] = a_project(h, 2)
        o[0] = a_values(s[0])
        attend(1)
        y[3] = a_project(h, 3)
        o[1] = a_values(s[1])
        attend(2)
        first = emit(0)
        rows = slice(0, first.shape[0])
        accum[rows, :] = first
        o[2] = a_values(s[2])
        attend(3)
        accum[rows, :] += emit(1)
        o[3] = a_values(s[3])
        accum[rows, :] += emit(2)
        last = emit(3)
        out = accum[rows, :] + last
        filler()
        return sum(y, []), sum(o, []), out

    def b_attention(t0):
        base = pl.ds(pl.multiple_of(t0, SEG), HALO + SEG)
        lane = lax.broadcasted_iota(jnp.int32, (SEG, 128), 1)
        pos = lax.broadcasted_iota(jnp.int32, (SEG, 128), 0) + t0

        def window(j, w):
            return qkvb.at[j, base][HALO - w * DIL:HALO - w * DIL + SEG, :]

        def exchange_sum(x, v):
            return x + jnp.where((lane & v) == 0, pltpu.roll(x, 128 - v, 1), pltpu.roll(x, v, 1))

        q = [window(j, 0) for j in range(NT)]
        logits = []
        for w in range(WIN):
            acc = q[0] * window(NT, w)
            for j in range(1, NT):
                acc = acc + q[j] * window(NT + j, w)
            acc = exchange_sum(exchange_sum(acc, 16), 1) * (DHB ** -0.5 * LOG2E)
            logits.append(jnp.where(pos >= w * DIL, acc, NEG * LOG2E) if w else acc)
        top = functools.reduce(jnp.maximum, logits)
        e = [jnp.exp2(x - top) for x in logits]
        inv = _reciprocal(functools.reduce(jnp.add, e))
        p = [x * inv for x in e]
        out = []
        for j in range(NT):
            acc = p[0] * window(2 * NT + j, 0)
            for w in range(1, WIN):
                acc = acc + p[w] * window(2 * NT + j, w)
            out.append(acc)
        return jnp.concatenate(out, axis=1).astype(BF16)

    def step(i, mem):
        slot = i % 2
        t0 = i * STEP

        @pl.when(i >= 2)
        def _():
            out_copy(i - 2, slot).wait()

        @pl.when(i == XA_HEAD // STEP)
        def _():
            wait_next_batch()

        def b_block(k):
            o = b_attention(t0 + k * SEG)
            ostage[slot, k * SEG:(k + 1) * SEG, D:2 * D] = _dot(o, b_out_weight()).astype(BF16)

        x = xa[pl.ds(pl.multiple_of(t0, STEP), STEP), :].astype(F32)

        h = jnp.concatenate([mem, x[:SEG + 8]], axis=0).astype(BF16)
        y0, o0, out0 = a_segment(
            h, lambda head, y: y[:L], lambda head, o: o[:L - 8], functools.partial(b_block, 0))
        ostage[slot, 0:SEG - 8, 0:D] = out0[NMEM:].astype(BF16)

        h = jnp.concatenate([out0[:NMEM], x[SEG + 8:]], axis=0).astype(BF16)
        _, _, out1 = a_segment(
            h,
            lambda head, y: jnp.concatenate([y[:NMEM], y0[head][L:], y[NMEM:]], axis=0),
            lambda head, o: jnp.concatenate([o[:NMEM], o0[head][L - 8:], o[NMEM:]], axis=0),
            functools.partial(b_block, 1))
        ostage[slot, SEG - 8:STEP, 0:D] = out1[NMEM:].astype(BF16)

        out_copy(i, slot).start()
        return out1[:NMEM]

    steps = S // STEP
    lax.fori_loop(0, steps, step, mem0_ref[...].astype(F32))
    for i in (steps - 2, steps - 1):
        out_copy(i, i % 2).wait()


def _word_rows(n):
    return pltpu.VMEM((-(-n // 64) * 64, 128), U32)


@functools.partial(jax.jit, static_argnames=("A_seg_len",))
def pallas_concat_heads__memory_aug_recurrent_mem_tr__sliding_local_dilated__prompt_kernel(
    A_x, A_mem0, A_Wq, A_Wk, A_Wv, A_Wo, A_seg_len, B_x, B_wqkv, B_wo,
):
    assert A_seg_len == SEG and A_x.shape == (1, S, D) and A_mem0.shape == (1, NMEM, D)
    assert A_Wq.shape == (D, HA, DHA) and B_x.shape == (1, S, D)
    hbm = pl.BlockSpec(memory_space=pl.ANY)
    grouped = (D // 16, 16 * HA, DHA)
    out = pl.pallas_call(
        _kernel,
        out_shape=jax.ShapeDtypeStruct((S, 2 * D), BF16),
        in_specs=[hbm, pl.BlockSpec(memory_space=pltpu.VMEM)] + [hbm] * 7,
        out_specs=hbm,
        scratch_shapes=[
            _word_rows((3 * HA + 1) * PITCH_A),
            pltpu.VMEM((NT, HA * DHA, 128), BF16),
            pltpu.VMEM((3, D // 2, D), U32),
            _word_rows((8 * NT + 1) * PITCH_B),
            *[pltpu.VMEM((3, hi - lo) + grouped[1:], BF16)
              for lo, hi in zip(A_SPLIT, A_SPLIT[1:])],
            pltpu.VMEM((D, 3 * D), BF16),
            pltpu.VMEM((NT, D, 128), BF16),
            pltpu.VMEM((3 * NT, HALO + S, 128), F32),
            pltpu.VMEM((S, D), BF16),
            pltpu.VMEM((S, D), BF16),
            pltpu.VMEM((2, STEP, 2 * D), BF16),
            pltpu.VMEM((NMEM + SEG + 8, D), F32),
            pltpu.SemaphoreType.DMA((len(K_SPLIT) + 7,)),
            pltpu.SemaphoreType.DMA((2,)),
        ],
        compiler_params=pltpu.CompilerParams(vmem_limit_bytes=120 * 1024 * 1024),
    )(
        A_x.reshape(S, D), A_mem0.reshape(NMEM, D),
        A_Wq.reshape(grouped), A_Wk.reshape(grouped), A_Wv.reshape(grouped),
        A_Wo.reshape(HA * DHA, D),
        B_x.reshape(S, D), B_wqkv, B_wo,
    )
    return out.reshape(1, S, 2 * D)
```
